```python
import os as _os
_os.environ.setdefault("JAX_PLATFORMS", "cpu")
import jax
import jax.numpy as jnp

def _softmax(x, axis=-1):
    return jax.nn.softmax(x, axis=axis)
def _gelu(x):
    return jax.nn.gelu(x, approximate=True)
def _silu(x):
    return jax.nn.silu(x)
def _sigmoid(x):
    return jax.nn.sigmoid(x)
def _layernorm(x, axis=-1, eps=1e-5):
    m = jnp.mean(x, axis=axis, keepdims=True)
    v = jnp.var(x, axis=axis, keepdims=True)
    return (x - m) / jnp.sqrt(v + eps)
def _scatter_add(tgt, idx, src, axis=0):
    return tgt.at[idx].add(src)
def _segment_sum(src, seg, n):
    return jax.ops.segment_sum(src, seg, n)
class _Rng:
    def __init__(self, key):
        self._k = key
    def _next(self):
        self._k, sub = jax.random.split(self._k)
        return sub
    def normal(self, shape):
        return jax.random.normal(self._next(), shape, dtype=jnp.bfloat16)
    def randint(self, lo, hi, shape):
        return jax.random.randint(self._next(), shape, lo, hi, dtype=jnp.int32)
    def uniform(self, shape, lo=0.0, hi=1.0):
        return jax.random.uniform(self._next(), shape, jnp.bfloat16, lo, hi)
    def permutation(self, n):
        return jax.random.permutation(self._next(), n)


kernel_name = 'gated_mix__grouped_kv_mqa__ssm_conv_s5__prompt'

def setup_inputs():
    _rng = _Rng(jax.random.key(int.from_bytes(__import__("os").urandom(4), "little")))
    _w = (lambda a: (lambda t: t.astype(jnp.bfloat16) if jnp.issubdtype(t.dtype, jnp.floating) else t)(jnp.asarray(a)))
    def _A_setup():
        B, S, D, H = 1, 2048, 512, 32
        Dh = D // H
        return {
            "x": _w((lambda *s: _rng.normal(s) * 0.05)(B, S, D)),
            "wq": _w((lambda *s: _rng.normal(s) * 1.6)(D, H * Dh)),
            "wk": _w((lambda *s: _rng.normal(s) * 1.6)(D, Dh)),
            "wv": _w((lambda *s: _rng.normal(s) * 0.05)(D, Dh)),
            "wo": _w((lambda *s: _rng.normal(s) * 0.05)(H * Dh, D)),
        }
    _A_in = _A_setup()

    def _B_setup():
        B, S, D = 1, 2048, 512
        P = D
        Lambda_re = -0.5 * jnp.exp((lambda *s: _rng.normal(s) * 0.4)(P))
        Lambda_im = (lambda *s: _rng.normal(s) * 0.4)(P) * 1.0
        B_re = (lambda *s: _rng.normal(s) * 0.4)(P, D) * (D ** -0.5)
        B_im = (lambda *s: _rng.normal(s) * 0.4)(P, D) * (D ** -0.5)
        C_re = (lambda *s: _rng.normal(s) * 0.4)(D, P) * (P ** -0.5)
        C_im = (lambda *s: _rng.normal(s) * 0.4)(D, P) * (P ** -0.5)
        log_dt = (lambda *s: _rng.normal(s) * 0.4)(P) * 0.3 - 2.0
        Dskip = (lambda *s: _rng.normal(s) * 0.4)(D)
        return {
            "x": _w((lambda *s: _rng.normal(s) * 0.05)(B, S, D)),
            "Lambda_re": _w(Lambda_re),
            "Lambda_im": _w(Lambda_im),
            "B_re": _w(B_re),
            "B_im": _w(B_im),
            "C_re": _w(C_re),
            "C_im": _w(C_im),
            "log_dt": _w(log_dt),
            "Dskip": _w(Dskip),
        }
    _B_in = _B_setup()

    return {
        "A_x": _A_in["x"],
        "A_wq": _A_in["wq"],
        "A_wk": _A_in["wk"],
        "A_wv": _A_in["wv"],
        "A_wo": _A_in["wo"],
        "B_x": _B_in["x"],
        "B_Lambda_re": _B_in["Lambda_re"],
        "B_Lambda_im": _B_in["Lambda_im"],
        "B_B_re": _B_in["B_re"],
        "B_B_im": _B_in["B_im"],
        "B_C_re": _B_in["C_re"],
        "B_C_im": _B_in["C_im"],
        "B_log_dt": _B_in["log_dt"],
        "B_Dskip": _B_in["Dskip"],
        "gate_w": _w((lambda *s: _rng.normal(s) * 0.05)(512) * 16.0),
    }

def reference(A_x, A_wq, A_wk, A_wv, A_wo, B_x, B_Lambda_re, B_Lambda_im, B_B_re, B_B_im, B_C_re, B_C_im, B_log_dt, B_Dskip, gate_w):
    def _A_ref(x, wq, wk, wv, wo):
        B, S, D = x.shape
        H = 32
        Dh = D // H
        q = (lambda x, *d: x.transpose(*d))((x @ wq).reshape(B, S, H, Dh), 0, 2, 1, 3)
        k = x @ wk
        v = x @ wv
        scores = jnp.einsum("bhqd,bkd->bhqk", q, k) * (Dh ** -0.5)
        p = _softmax(scores, axis=-1)
        o = jnp.einsum("bhqk,bkd->bhqd", p, v)
        return (lambda x, *d: x.transpose(*d))(o, 0, 2, 1, 3).reshape(B, S, H * Dh) @ wo

    def _B_ref(x, Lambda_re, Lambda_im, B_re, B_im, C_re, C_im, log_dt, Dskip):
        Bsz, L, H = x.shape
        Lam = Lambda_re + 1j * Lambda_im
        Bmat = B_re + 1j * B_im
        Cmat = C_re + 1j * C_im
        dt = jnp.exp(log_dt)
        Lam_bar = jnp.exp(dt * Lam)
        B_bar = ((Lam_bar - 1.0) / Lam)[:, None] * Bmat
        Bu = jnp.einsum("bld,pd->blp", x + 0j, B_bar)
        h = jnp.zeros_like(Bu[:, 0, :])
        hs = []
        for t in range(L):
            h = Lam_bar[None, :] * h + Bu[:, t, :]
            hs.append(h)
        hseq = jnp.stack(hs, 1)
        y = 2.0 * jnp.einsum("blp,dp->bld", hseq, Cmat).real + x * Dskip[None, None, :]
        return y

    x = A_x
    g = _sigmoid((x * gate_w).sum(-1, keepdims=True))
    a = _A_ref(x, A_wq, A_wk, A_wv, A_wo)
    b = _B_ref(x, B_Lambda_re, B_Lambda_im, B_B_re, B_B_im, B_C_re, B_C_im, B_log_dt, B_Dskip)
    return g * a + (1 - g) * b
```

```python
import functools
import jax
import jax.numpy as jnp
from jax import lax
import jax.experimental.pallas as pl
import jax.experimental.pallas.tpu as pltpu

S = 2048
D = 512
H = 32
DH = 16
P = 512
TS = 256
TK = 128
NH = 4
f32 = jnp.float32
bf16 = jnp.bfloat16

NT = (((1,), (1,)), ((), ()))
TN = (((0,), (0,)), ((), ()))


def _cmul(ar, ai, br, bi):
    return ar * br - ai * bi, ar * bi + ai * br


def _kernel(x_ref, wqT_ref, wk_ref, wvT_ref, wo_ref, bcat_ref, cre_ref, cim_ref, vec_ref,
            o_ref, k_s, vt_s, qa_s, ot_s, cu_s, ch_s):
    i = pl.program_id(0)

    @pl.when(i == 0)
    def _init():
        x = x_ref[...]
        k_s[...] = jnp.dot(x, wk_ref[...], preferred_element_type=f32).astype(bf16)
        vt_s[...] = lax.dot_general(wvT_ref[...], x, NT, preferred_element_type=f32).astype(bf16)
        cu_s[...] = jnp.zeros_like(cu_s)
        ch_s[...] = jnp.zeros_like(ch_s)

    row0 = pl.multiple_of(i * TS, TS)
    xb = x_ref[pl.ds(row0, TS), :]

    qt = (lax.dot_general(wqT_ref[...], xb, NT, preferred_element_type=f32) * 0.25).astype(bf16)
    for b_ in range(H // NH):
        qa_s[b_] = jnp.concatenate(
            [qt[(b_ * NH + j) * DH:(b_ * NH + j + 1) * DH, :] for j in range(NH)], axis=1)

    def blk(b, carry):
        q = qa_s[b]
        nl = NH * TS
        n = S // TK
        s = jnp.dot(k_s[0:TK, :], q, preferred_element_type=f32)
        m = jnp.max(s, axis=0, keepdims=True)
        p = jnp.exp(s - m)
        l = jnp.sum(p.reshape(TK // 8, 8, nl), axis=0)
        pb = p.astype(bf16)
        acc = jnp.zeros((DH, nl), f32)
        for c in range(1, n):
            s = jnp.dot(k_s[c * TK:(c + 1) * TK, :], q, preferred_element_type=f32)
            acc = acc + jnp.dot(vt_s[:, (c - 1) * TK:c * TK], pb, preferred_element_type=f32)
            m_new = jnp.maximum(m, jnp.max(s, axis=0, keepdims=True))
            alpha = jnp.exp(m - m_new)
            p = jnp.exp(s - m_new)
            l = alpha * l + jnp.sum(p.reshape(TK // 8, 8, nl), axis=0)
            acc = alpha * acc
            pb = p.astype(bf16)
            m = m_new
        acc = acc + jnp.dot(vt_s[:, (n - 1) * TK:n * TK], pb, preferred_element_type=f32)
        lsum = jnp.sum(l, axis=0, keepdims=True)
        ob = (acc / lsum).astype(bf16)
        for j in range(NH):
            hr = pl.multiple_of((b * NH + j) * DH, DH)
            ot_s[pl.ds(hr, DH), :] = ob[:, j * TS:(j + 1) * TS]
        return carry

    lax.fori_loop(0, H // NH, blk, 0)

    a = lax.dot_general(ot_s[...], wo_ref[...], TN, preferred_element_type=f32)

    lre = vec_ref[0:1, :]
    lim = vec_ref[1:2, :]
    ldt = vec_ref[2:3, :]
    dsk = vec_ref[3:4, :]
    gw = vec_ref[4:5, :]
    dt = jnp.exp(ldt).astype(bf16).astype(f32)
    er = jnp.exp(dt * lre)
    ang = dt * lim
    l1r = er * jnp.cos(ang)
    l1i = er * jnp.sin(ang)
    den = lre * lre + lim * lim
    nr = l1r - 1.0
    ni = l1i
    cfr = (nr * lre + ni * lim) / den
    cfi = (ni * lre - nr * lim) / den
    l2r, l2i = _cmul(l1r, l1i, l1r, l1i)
    l4r, l4i = _cmul(l2r, l2i, l2r, l2i)
    l8r, l8i = _cmul(l4r, l4i, l4r, l4i)

    bu = lax.dot_general(xb, bcat_ref[...], NT, preferred_element_type=f32)
    br = bu[:, :P]
    bi = bu[:, P:]
    ur, ui = _cmul(br, bi, cfr, cfi)

    uer = jnp.concatenate([cu_s[0], ur], axis=0)
    uei = jnp.concatenate([cu_s[1], ui], axis=0)
    cu_s[0] = ur[TS - 8:, :]
    cu_s[1] = ui[TS - 8:, :]

    def stage(xr, xi, sh, cr, ci):
        sr = pltpu.roll(xr, sh, 0)
        si = pltpu.roll(xi, sh, 0)
        tr, ti = _cmul(sr, si, cr, ci)
        return xr + tr, xi + ti

    u1r, u1i = stage(uer, uei, 1, l1r, l1i)
    u2r, u2i = stage(u1r, u1i, 2, l2r, l2i)
    u3r, u3i = stage(u2r, u2i, 4, l4r, l4i)
    u3r = u3r[8:, :]
    u3i = u3i[8:, :]

    hr_prev = ch_s[0]
    hi_prev = ch_s[1]
    hrs = []
    his = []
    for j in range(TS // 8):
        tr, ti = _cmul(hr_prev, hi_prev, l8r, l8i)
        hr_prev = u3r[j * 8:(j + 1) * 8, :] + tr
        hi_prev = u3i[j * 8:(j + 1) * 8, :] + ti
        hrs.append(hr_prev)
        his.append(hi_prev)
    ch_s[0] = hr_prev
    ch_s[1] = hi_prev
    hre = jnp.concatenate(hrs, axis=0).astype(bf16)
    him = jnp.concatenate(his, axis=0).astype(bf16)
    y = lax.dot_general(hre, cre_ref[...], NT, preferred_element_type=f32) - \
        lax.dot_general(him, cim_ref[...], NT, preferred_element_type=f32)
    xf = xb.astype(f32)
    b = 2.0 * y + (xf * dsk).astype(bf16).astype(f32)

    gl = jnp.sum(xf * gw, axis=-1, keepdims=True)
    g = jax.nn.sigmoid(gl)
    o_ref[...] = g * a + (1.0 - g) * b


@jax.jit
def pallas_gated_mix__grouped_kv_mqa__ssm_conv_s5__prompt_kernel(
    A_x, A_wq, A_wk, A_wv, A_wo, B_x, B_Lambda_re, B_Lambda_im, B_B_re, B_B_im,
    B_C_re, B_C_im, B_log_dt, B_Dskip, gate_w,
):
    del B_x
    x2 = A_x.reshape(S, D)
    wqT = A_wq.T
    wvT = A_wv.T
    bcat = jnp.concatenate([B_B_re, B_B_im], axis=0)
    zero = jnp.zeros((3, D), bf16)
    vec = jnp.concatenate([B_Lambda_re[None], B_Lambda_im[None], B_log_dt[None], B_Dskip[None],
                           gate_w[None], zero], axis=0).astype(f32)
    full = lambda shp: pl.BlockSpec(shp, lambda i: (0,) * len(shp))
    out = pl.pallas_call(
        _kernel,
        grid=(S // TS,),
        in_specs=[full((S, D)), full((D, D)), full((D, DH)), full((DH, D)), full((D, D)),
                  full((2 * P, D)), full((D, P)), full((D, P)), full((8, D))],
        out_specs=pl.BlockSpec((TS, D), lambda i: (i, 0)),
        out_shape=jax.ShapeDtypeStruct((S, D), f32),
        scratch_shapes=[
            pltpu.VMEM((S, DH), bf16),
            pltpu.VMEM((DH, S), bf16),
            pltpu.VMEM((H // NH, DH, NH * TS), bf16),
            pltpu.VMEM((D, TS), bf16),
            pltpu.VMEM((2, 8, P), f32),
            pltpu.VMEM((2, 8, P), f32),
        ],
        compiler_params=pltpu.CompilerParams(
            dimension_semantics=("arbitrary",),
            vmem_limit_bytes=100 * 1024 * 1024,
        ),
    )(x2, wqT, A_wk, wvT, A_wo, bcat, B_C_re, B_C_im, vec)
    return out.reshape(1, S, D)
```

```python
import functools
import jax
import jax.numpy as jnp
from jax import lax
import jax.experimental.pallas as pl
import jax.experimental.pallas.tpu as pltpu

S = 2048
D = 512
H = 32
DH = 16
P = 512
TS = 256
TK = 128
NH = 4
LW = 256
f32 = jnp.float32
bf16 = jnp.bfloat16

NT = (((1,), (1,)), ((), ()))
TN = (((0,), (0,)), ((), ()))


def _cmul(ar, ai, br, bi):
    return ar * br - ai * bi, ar * bi + ai * br


def _kernel(x_ref, wqT_ref, wk_ref, wvT_ref, wo_ref, bcat_ref, cre_ref, cim_ref, vec_ref,
            o_ref, k_s, vt_s, qa_s, ot_s, cu_s, ch_s):
    i = pl.program_id(0)

    @pl.when(i == 0)
    def _init():
        x = x_ref[...]
        k_s[...] = jnp.dot(x, wk_ref[...], preferred_element_type=f32).astype(bf16)
        vt_s[...] = lax.dot_general(wvT_ref[...], x, NT, preferred_element_type=f32).astype(bf16)
        cu_s[...] = jnp.zeros_like(cu_s)
        ch_s[...] = jnp.zeros_like(ch_s)

    row0 = pl.multiple_of(i * TS, TS)
    xb = x_ref[pl.ds(row0, TS), :]

    qt = (lax.dot_general(wqT_ref[...], xb, NT, preferred_element_type=f32) * 0.25).astype(bf16)
    for b_ in range(H // NH):
        qa_s[b_] = jnp.concatenate(
            [qt[(b_ * NH + j) * DH:(b_ * NH + j + 1) * DH, :] for j in range(NH)], axis=1)

    def blk(b, carry):
        n = S // TK
        nt = (NH * TS) // LW
        st = []
        for j in range(nt):
            q = qa_s[b, :, j * LW:(j + 1) * LW]
            s = jnp.dot(k_s[0:TK, :], q, preferred_element_type=f32)
            m = jnp.max(s, axis=0, keepdims=True)
            p = jnp.exp(s - m)
            l = jnp.sum(p.reshape(TK // 8, 8, LW), axis=0)
            st.append((q, m, l, p.astype(bf16), jnp.zeros((DH, LW), f32)))
        for c in range(1, n):
            for j in range(nt):
                q, m, l, pb, acc = st[j]
                s = jnp.dot(k_s[c * TK:(c + 1) * TK, :], q, preferred_element_type=f32)
                acc = acc + jnp.dot(vt_s[:, (c - 1) * TK:c * TK], pb, preferred_element_type=f32)
                m_new = jnp.maximum(m, jnp.max(s, axis=0, keepdims=True))
                alpha = jnp.exp(m - m_new)
                p = jnp.exp(s - m_new)
                l = alpha * l + jnp.sum(p.reshape(TK // 8, 8, LW), axis=0)
                st[j] = (q, m_new, l, p.astype(bf16), alpha * acc)
        for j in range(nt):
            q, m, l, pb, acc = st[j]
            acc = acc + jnp.dot(vt_s[:, (n - 1) * TK:n * TK], pb, preferred_element_type=f32)
            lsum = jnp.sum(l, axis=0, keepdims=True)
            ob = (acc / lsum).astype(bf16)
            for t in range(LW // min(LW, TS)):
                lane0 = j * LW + t * min(LW, TS)
                hh = lane0 // TS
                off = lane0 % TS
                w = min(LW, TS)
                hr = pl.multiple_of((b * NH + hh) * DH, DH)
                ot_s[pl.ds(hr, DH), off:off + w] = ob[:, t * w:(t + 1) * w]
        return carry

    lax.fori_loop(0, H // NH, blk, 0)

    a = lax.dot_general(ot_s[...], wo_ref[...], TN, preferred_element_type=f32)

    lre = vec_ref[0:1, :]
    lim = vec_ref[1:2, :]
    ldt = vec_ref[2:3, :]
    dsk = vec_ref[3:4, :]
    gw = vec_ref[4:5, :]
    dt = jnp.exp(ldt).astype(bf16).astype(f32)
    er = jnp.exp(dt * lre)
    ang = dt * lim
    l1r = er * jnp.cos(ang)
    l1i = er * jnp.sin(ang)
    den = lre * lre + lim * lim
    nr = l1r - 1.0
    ni = l1i
    cfr = (nr * lre + ni * lim) / den
    cfi = (ni * lre - nr * lim) / den
    l2r, l2i = _cmul(l1r, l1i, l1r, l1i)
    l4r, l4i = _cmul(l2r, l2i, l2r, l2i)
    l8r, l8i = _cmul(l4r, l4i, l4r, l4i)

    bu = lax.dot_general(xb, bcat_ref[...], NT, preferred_element_type=f32)
    br = bu[:, :P]
    bi = bu[:, P:]
    ur, ui = _cmul(br, bi, cfr, cfi)

    uer = jnp.concatenate([cu_s[0], ur], axis=0)
    uei = jnp.concatenate([cu_s[1], ui], axis=0)
    cu_s[0] = ur[TS - 8:, :]
    cu_s[1] = ui[TS - 8:, :]

    def stage(xr, xi, sh, cr, ci):
        sr = pltpu.roll(xr, sh, 0)
        si = pltpu.roll(xi, sh, 0)
        tr, ti = _cmul(sr, si, cr, ci)
        return xr + tr, xi + ti

    u1r, u1i = stage(uer, uei, 1, l1r, l1i)
    u2r, u2i = stage(u1r, u1i, 2, l2r, l2i)
    u3r, u3i = stage(u2r, u2i, 4, l4r, l4i)
    u3r = u3r[8:, :]
    u3i = u3i[8:, :]

    hr_prev = ch_s[0]
    hi_prev = ch_s[1]
    hrs = []
    his = []
    for j in range(TS // 8):
        tr, ti = _cmul(hr_prev, hi_prev, l8r, l8i)
        hr_prev = u3r[j * 8:(j + 1) * 8, :] + tr
        hi_prev = u3i[j * 8:(j + 1) * 8, :] + ti
        hrs.append(hr_prev)
        his.append(hi_prev)
    ch_s[0] = hr_prev
    ch_s[1] = hi_prev
    hre = jnp.concatenate(hrs, axis=0).astype(bf16)
    him = jnp.concatenate(his, axis=0).astype(bf16)
    y = lax.dot_general(hre, cre_ref[...], NT, preferred_element_type=f32) - \
        lax.dot_general(him, cim_ref[...], NT, preferred_element_type=f32)
    xf = xb.astype(f32)
    b = 2.0 * y + (xf * dsk).astype(bf16).astype(f32)

    gl = jnp.sum(xf * gw, axis=-1, keepdims=True)
    g = jax.nn.sigmoid(gl)
    o_ref[...] = g * a + (1.0 - g) * b


@jax.jit
def pallas_gated_mix__grouped_kv_mqa__ssm_conv_s5__prompt_kernel(
    A_x, A_wq, A_wk, A_wv, A_wo, B_x, B_Lambda_re, B_Lambda_im, B_B_re, B_B_im,
    B_C_re, B_C_im, B_log_dt, B_Dskip, gate_w,
):
    del B_x
    x2 = A_x.reshape(S, D)
    wqT = A_wq.T
    wvT = A_wv.T
    bcat = jnp.concatenate([B_B_re, B_B_im], axis=0)
    zero = jnp.zeros((3, D), bf16)
    vec = jnp.concatenate([B_Lambda_re[None], B_Lambda_im[None], B_log_dt[None], B_Dskip[None],
                           gate_w[None], zero], axis=0).astype(f32)
    full = lambda shp: pl.BlockSpec(shp, lambda i: (0,) * len(shp))
    out = pl.pallas_call(
        _kernel,
        grid=(S // TS,),
        in_specs=[full((S, D)), full((D, D)), full((D, DH)), full((DH, D)), full((D, D)),
                  full((2 * P, D)), full((D, P)), full((D, P)), full((8, D))],
        out_specs=pl.BlockSpec((TS, D), lambda i: (i, 0)),
        out_shape=jax.ShapeDtypeStruct((S, D), f32),
        scratch_shapes=[
            pltpu.VMEM((S, DH), bf16),
            pltpu.VMEM((DH, S), bf16),
            pltpu.VMEM((H // NH, DH, NH * TS), bf16),
            pltpu.VMEM((D, TS), bf16),
            pltpu.VMEM((2, 8, P), f32),
            pltpu.VMEM((2, 8, P), f32),
        ],
        compiler_params=pltpu.CompilerParams(
            dimension_semantics=("arbitrary",),
            vmem_limit_bytes=100 * 1024 * 1024,
        ),
    )(x2, wqT, A_wk, wvT, A_wo, bcat, B_C_re, B_C_im, vec)
    return out.reshape(1, S, D)
```

```python
import functools
import jax
import jax.numpy as jnp
from jax import lax
import jax.experimental.pallas as pl
import jax.experimental.pallas.tpu as pltpu

S = 2048
D = 512
H = 32
DH = 16
P = 512
TS = 256
TK = 128
NH = 4
LW = 256
f32 = jnp.float32
bf16 = jnp.bfloat16

NT = (((1,), (1,)), ((), ()))
TN = (((0,), (0,)), ((), ()))


def _cmul(ar, ai, br, bi):
    return ar * br - ai * bi, ar * bi + ai * br


def _kernel(x_ref, wqT_ref, wk_ref, wvT_ref, wo_ref, bcat_ref, cre_ref, cim_ref, vec_ref,
            o_ref, k_s, vt_s, qa_s, ot_s, cu_s, ch_s):
    i = pl.program_id(0)

    @pl.when(i == 0)
    def _init():
        x = x_ref[...]
        k_s[...] = jnp.dot(x, wk_ref[...], preferred_element_type=f32).astype(bf16)
        vt_s[...] = lax.dot_general(wvT_ref[...], x, NT, preferred_element_type=f32).astype(bf16)
        cu_s[...] = jnp.zeros_like(cu_s)
        ch_s[...] = jnp.zeros_like(ch_s)

    row0 = pl.multiple_of(i * TS, TS)
    xb = x_ref[pl.ds(row0, TS), :]

    lre = vec_ref[0:1, :]
    lim = vec_ref[1:2, :]
    ldt = vec_ref[2:3, :]
    dsk = vec_ref[3:4, :]
    gw = vec_ref[4:5, :]
    dt = jnp.exp(ldt).astype(bf16).astype(f32)
    er = jnp.exp(dt * lre)
    ang = dt * lim
    l1r = er * jnp.cos(ang)
    l1i = er * jnp.sin(ang)
    den = lre * lre + lim * lim
    nr = l1r - 1.0
    ni = l1i
    cfr = (nr * lre + ni * lim) / den
    cfi = (ni * lre - nr * lim) / den
    l2r, l2i = _cmul(l1r, l1i, l1r, l1i)
    l4r, l4i = _cmul(l2r, l2i, l2r, l2i)
    l8r, l8i = _cmul(l4r, l4i, l4r, l4i)

    bu = lax.dot_general(xb, bcat_ref[...], NT, preferred_element_type=f32)
    br = bu[:, :P]
    bi = bu[:, P:]
    ur, ui = _cmul(br, bi, cfr, cfi)

    uer = jnp.concatenate([cu_s[0], ur], axis=0)
    uei = jnp.concatenate([cu_s[1], ui], axis=0)
    cu_s[0] = ur[TS - 8:, :]
    cu_s[1] = ui[TS - 8:, :]

    def stage(xr, xi, sh, cr, ci):
        sr = pltpu.roll(xr, sh, 0)
        si = pltpu.roll(xi, sh, 0)
        tr, ti = _cmul(sr, si, cr, ci)
        return xr + tr, xi + ti

    u1r, u1i = stage(uer, uei, 1, l1r, l1i)
    u2r, u2i = stage(u1r, u1i, 2, l2r, l2i)
    u3r, u3i = stage(u2r, u2i, 4, l4r, l4i)
    u3r = u3r[8:, :]
    u3i = u3i[8:, :]

    hr_prev = ch_s[0]
    hi_prev = ch_s[1]
    hrs = []
    his = []
    for j in range(TS // 8):
        tr, ti = _cmul(hr_prev, hi_prev, l8r, l8i)
        hr_prev = u3r[j * 8:(j + 1) * 8, :] + tr
        hi_prev = u3i[j * 8:(j + 1) * 8, :] + ti
        hrs.append(hr_prev)
        his.append(hi_prev)
    ch_s[0] = hr_prev
    ch_s[1] = hi_prev
    hre = jnp.concatenate(hrs, axis=0).astype(bf16)
    him = jnp.concatenate(his, axis=0).astype(bf16)
    y = lax.dot_general(hre, cre_ref[...], NT, preferred_element_type=f32) - \
        lax.dot_general(him, cim_ref[...], NT, preferred_element_type=f32)
    xf = xb.astype(f32)
    b = 2.0 * y + (xf * dsk).astype(bf16).astype(f32)

    qt = (lax.dot_general(wqT_ref[...], xb, NT, preferred_element_type=f32) * 0.25).astype(bf16)
    for b_ in range(H // NH):
        qa_s[b_] = jnp.concatenate(
            [qt[(b_ * NH + j) * DH:(b_ * NH + j + 1) * DH, :] for j in range(NH)], axis=1)

    n = S // TK
    nt = (NH * TS) // LW
    w = min(LW, TS)

    def finalize(lb, j, acc, l):
        lsum = jnp.sum(l, axis=0, keepdims=True)
        ob = (acc / lsum).astype(bf16)
        for t in range(LW // w):
            lane0 = j * LW + t * w
            hr = (lb * NH + lane0 // TS) * DH
            off = lane0 % TS
            ot_s[hr:hr + DH, off:off + w] = ob[:, t * w:(t + 1) * w]

    st = [None] * nt
    pend = None
    for gi in range((H // NH) * n + 1):
        lb, c = divmod(gi, n)
        live = gi < (H // NH) * n
        for j in range(nt):
            if live:
                if c == 0:
                    q = qa_s[lb, :, j * LW:(j + 1) * LW]
                else:
                    q = st[j][0]
                s = jnp.dot(k_s[c * TK:(c + 1) * TK, :], q, preferred_element_type=f32)
            if pend is not None:
                pb_, pc_, pbs = pend
                q_, m_, l_, acc_ = st[j]
                acc_ = acc_ + jnp.dot(vt_s[:, pc_ * TK:(pc_ + 1) * TK], pbs[j],
                                      preferred_element_type=f32)
                if pc_ == n - 1:
                    finalize(pb_, j, acc_, l_)
                else:
                    st[j] = (q_, m_, l_, acc_)
            if live:
                if c == 0:
                    m = jnp.max(s, axis=0, keepdims=True)
                    p = jnp.exp(s - m)
                    l = jnp.sum(p.reshape(TK // 8, 8, LW), axis=0)
                    st[j] = (q, m, l, jnp.zeros((DH, LW), f32))
                else:
                    q, m, l, acc = st[j]
                    m_new = jnp.maximum(m, jnp.max(s, axis=0, keepdims=True))
                    alpha = jnp.exp(m - m_new)
                    p = jnp.exp(s - m_new)
                    l = alpha * l + jnp.sum(p.reshape(TK // 8, 8, LW), axis=0)
                    st[j] = (q, m_new, l, alpha * acc)
                if j == 0:
                    pbs_new = []
                pbs_new.append(p.astype(bf16))
        pend = (lb, c, pbs_new) if live else None

    a = lax.dot_general(ot_s[...], wo_ref[...], TN, preferred_element_type=f32)

    gl = jnp.sum(xf * gw, axis=-1, keepdims=True)
    g = jax.nn.sigmoid(gl)
    o_ref[...] = g * a + (1.0 - g) * b


@jax.jit
def pallas_gated_mix__grouped_kv_mqa__ssm_conv_s5__prompt_kernel(
    A_x, A_wq, A_wk, A_wv, A_wo, B_x, B_Lambda_re, B_Lambda_im, B_B_re, B_B_im,
    B_C_re, B_C_im, B_log_dt, B_Dskip, gate_w,
):
    del B_x
    x2 = A_x.reshape(S, D)
    wqT = A_wq.T
    wvT = A_wv.T
    bcat = jnp.concatenate([B_B_re, B_B_im], axis=0)
    zero = jnp.zeros((3, D), bf16)
    vec = jnp.concatenate([B_Lambda_re[None], B_Lambda_im[None], B_log_dt[None], B_Dskip[None],
                           gate_w[None], zero], axis=0).astype(f32)
    full = lambda shp: pl.BlockSpec(shp, lambda i: (0,) * len(shp))
    out = pl.pallas_call(
        _kernel,
        grid=(S // TS,),
        in_specs=[full((S, D)), full((D, D)), full((D, DH)), full((DH, D)), full((D, D)),
                  full((2 * P, D)), full((D, P)), full((D, P)), full((8, D))],
        out_specs=pl.BlockSpec((TS, D), lambda i: (i, 0)),
        out_shape=jax.ShapeDtypeStruct((S, D), f32),
        scratch_shapes=[
            pltpu.VMEM((S, DH), bf16),
            pltpu.VMEM((DH, S), bf16),
            pltpu.VMEM((H // NH, DH, NH * TS), bf16),
            pltpu.VMEM((D, TS), bf16),
            pltpu.VMEM((2, 8, P), f32),
            pltpu.VMEM((2, 8, P), f32),
        ],
        compiler_params=pltpu.CompilerParams(
            dimension_semantics=("arbitrary",),
            vmem_limit_bytes=100 * 1024 * 1024,
        ),
    )(x2, wqT, A_wk, wvT, A_wo, bcat, B_C_re, B_C_im, vec)
    return out.reshape(1, S, D)
```
